```python
import jax
import jax.numpy as jnp

def _softmax(x, axis=-1):
    return jax.nn.softmax(x, axis=axis)
def _gelu(x):
    return jax.nn.gelu(x, approximate=True)
def _silu(x):
    return jax.nn.silu(x)
def _sigmoid(x):
    return jax.nn.sigmoid(x)
def _layernorm(x, axis=-1, eps=1e-5):
    m = jnp.mean(x, axis=axis, keepdims=True)
    v = jnp.var(x, axis=axis, keepdims=True)
    return (x - m) / jnp.sqrt(v + eps)
def _scatter_add(tgt, idx, src, axis=0):
    return tgt.at[idx].add(src)
def _segment_sum(src, seg, n):
    return jax.ops.segment_sum(src, seg, n)
class _Rng:
    def __init__(self, key):
        self._k = key
    def _next(self):
        self._k, sub = jax.random.split(self._k)
        return sub
    def normal(self, shape):
        return jax.random.normal(self._next(), shape, dtype=jnp.bfloat16)
    def randint(self, lo, hi, shape):
        return jax.random.randint(self._next(), shape, lo, hi, dtype=jnp.int32)
    def uniform(self, shape, lo=0.0, hi=1.0):
        return jax.random.uniform(self._next(), shape, jnp.bfloat16, lo, hi)
    def permutation(self, n):
        return jax.random.permutation(self._next(), n)


kernel_name = 'sequential_preLN__spectral_gfnet__swiglu_ffn__prompt'

def _fwd_setup_inputs():
    _rng = _Rng(jax.random.key(int.from_bytes(__import__("os").urandom(4), "little")))
    _w = (lambda a: (lambda t: t.astype(jnp.bfloat16) if jnp.issubdtype(t.dtype, jnp.floating) else t)(jnp.asarray(a)))
    def _A_setup():
        B, S, D = 1, 2048, 576
        Df = D // 2 + 1
        return {
            "x": _w((lambda *s: _rng.normal(s) * 0.05)(B, S, D)),
            "w_r": _w((lambda *s: _rng.normal(s) * 0.05)(S, Df) * 0.02),
            "w_i": _w((lambda *s: _rng.normal(s) * 0.05)(S, Df) * 0.02),
        }
    _A_in = _A_setup()

    def _B_setup():
        B, S, D, F = 1, 2048, 576, 4608
        return {
            "x": _w((lambda *s: _rng.normal(s) * 0.05)(B, S, D)),
            "w_gate": _w((lambda *s: _rng.normal(s) * 0.05)(D, F)),
            "w_up": _w((lambda *s: _rng.normal(s) * 0.05)(D, F)),
            "w_down": _w((lambda *s: _rng.normal(s) * 0.05)(F, D)),
        }
    _B_in = _B_setup()

    return {
        "A_x": _A_in["x"],
        "A_w_r": _A_in["w_r"],
        "A_w_i": _A_in["w_i"],
        "B_x": _B_in["x"],
        "B_w_gate": _B_in["w_gate"],
        "B_w_up": _B_in["w_up"],
        "B_w_down": _B_in["w_down"],
    }

def _fwd_reference(A_x, A_w_r, A_w_i, B_x, B_w_gate, B_w_up, B_w_down):
    def _A_ref(x, w_r, w_i):
        B, S, D = x.shape
        X = (lambda x, axes=(-2,-1): jnp.fft.rfft2(x.astype(jnp.float32), axes=axes))(x, axes=(-2, -1))
        W = w_r + 1j * w_i
        X = X * W
        y = (lambda x, s, axes=(-2,-1): jnp.fft.irfft2(x, s=s, axes=axes).astype(jnp.bfloat16))(X, (S, D), axes=(-2, -1))
        return y

    def _B_ref(x, w_gate, w_up, w_down):
        g = _silu(x @ w_gate)
        u = x @ w_up
        return (g * u) @ w_down

    x = A_x
    h = x + _A_ref(_layernorm(x, axis=-1), A_w_r, A_w_i)
    h2 = h + _B_ref(_layernorm(h, axis=-1), B_w_gate, B_w_up, B_w_down)
    return h2


def setup_inputs():
    _inp = _fwd_setup_inputs()
    _gk = jax.random.fold_in(jax.random.key(int.from_bytes(__import__("os").urandom(4), "little")), 2**31 - 1)
    _shapes = [[1, 2048, 576]]
    _dtypes = ['bfloat16']
    _gks = jax.random.split(_gk, len(_shapes))
    _gs = [jax.random.normal(k, s, dtype=jnp.dtype(d)) * 0.05 for k, s, d in zip(_gks, _shapes, _dtypes)]
    _inp["grad_out"] = _gs[0]
    return _inp

def reference(A_x, A_w_r, A_w_i, B_w_gate, B_w_up, B_w_down, B_x, grad_out):
    _const = dict(B_x=B_x)
    def _f(*_d):
        return _fwd_reference(**{'A_x': _d[0], 'A_w_r': _d[1], 'A_w_i': _d[2], 'B_w_gate': _d[3], 'B_w_up': _d[4], 'B_w_down': _d[5], **_const})
    _out, _vjp = jax.vjp(_f, A_x, A_w_r, A_w_i, B_w_gate, B_w_up, B_w_down)
    _grads = _vjp(grad_out)
    _out0 = jnp.asarray(_out)
    return (_out0, *[jnp.asarray(_g) for _g in _grads])
```

```python
from itertools import chain

import numpy as np
import jax
import jax.numpy as jnp
import jax.experimental.pallas as pl
import jax.experimental.pallas.tpu as pltpu

S, D, F = 2048, 576, 4608
DF = D // 2 + 1
DH = D // 2
NE, NO = 160, 144
R = NE + NO
BF = 512
NC, NG = F // BF, 4
Q = D // 4
EPS = 1e-5
f32, bf16, u32 = jnp.float32, jnp.bfloat16, jnp.uint32
NN = (((1,), (0,)), ((), ()))
NT = (((1,), (1,)), ((), ()))


def _tables():
    d = np.arange(DH)[None, :]
    ko = 2 * np.arange(NO)[:, None] + 1
    ce = np.zeros((2, NE, Q))
    for r in range(2):
        ke = np.arange(2 * r, DF, 4)[:, None]
        ang = 2 * np.pi * ((ke * d[:, :Q]) % D) / D
        ce[r, :ke.shape[0]] = np.cos(ang)
        ce[r, NE // 2:NE // 2 + ke.shape[0]] = -np.sin(ang)
    ang = 2 * np.pi * ((ko * d) % D) / D
    co = np.concatenate([np.cos(ang), -np.sin(ang)], 0)
    s2 = np.arange(128)[None, :, None]
    k = np.arange(16)[:, None, None] + 16 * np.arange(128)[None, None, :]
    ang = 2 * np.pi * ((s2 * k) % S) / S
    c, s = np.cos(ang), -np.sin(ang)
    g = np.concatenate([np.concatenate([c, s], 2), np.concatenate([-s, c], 2)], 1)
    t = lambda a: np.ascontiguousarray(a, dtype=np.float32).astype(bf16)
    g = t(g).view(np.uint16).astype(np.uint32).reshape(16 * 128, 2, 256)
    return t(ce), t(co), t(ce.transpose(0, 2, 1)), t(co.T), g[:, 0] | (g[:, 1] << 16)


_CE, _CO, _CET, _COT, _G = _tables()


def _dot(a, b, dn=NN):
    return jax.lax.dot_general(a, b, dn, preferred_element_type=f32)


def _fft4(x, sg):
    (ar, ai), (br, bi), (cr, ci), (dr, di) = x
    t0 = (ar + cr, ai + ci)
    t1 = (ar - cr, ai - ci)
    t2 = (br + dr, bi + di)
    t3 = (br - dr, bi - di)
    p = (t1[0] + t3[1], t1[1] - t3[0])
    m = (t1[0] - t3[1], t1[1] + t3[0])
    y1, y3 = (p, m) if sg < 0 else (m, p)
    return [(t0[0] + t2[0], t0[1] + t2[1]), y1, (t0[0] - t2[0], t0[1] - t2[1]), y3]


def _tw(x, e, sg):
    r, i = x
    if e == 0:
        return x
    c, s = float(np.cos(np.pi * e / 8)), sg * float(np.sin(np.pi * e / 8))
    if e == 4:
        return (i, -r) if sg < 0 else (-i, r)
    if e % 2 == 0:
        return ((r - i) * c, (r + i) * c) if c * s > 0 else ((r + i) * c, (i - r) * c)
    return (r * c - i * s, r * s + i * c)


def _fft16(x, sg):
    a = [_fft4(x[j::4], sg) for j in range(4)]
    out = [None] * 16
    for k in range(4):
        y = _fft4([_tw(a[j][k], j * k, sg) for j in range(4)], sg)
        for m in range(4):
            out[k + 4 * m] = y[m]
    return out


def _forms(x11, x12, x21, x22):
    return [x11 + x22, x21 + x22, x11, x22, x11 + x12, x21 - x11, x12 - x22]


_FORM = (((0, 1), (3, 1)), ((2, 1), (3, 1)), ((0, 1),), ((3, 1),), ((0, 1), (1, 1)),
         ((2, 1), (0, -1)), ((1, 1), (3, -1)))
_B2A = (0, 2, 6, 5, 3, 4, 1)
_B2A2 = [7 * _B2A[t] + _B2A[u] for t in range(7) for u in range(7)]
_ORDER = (2, 4, 1, 3, 0, 5, 6)
_INTO = (((0, 1), (3, 1)), ((2, 1), (3, -1)), ((1, 1), (3, 1)), ((2, 1), (0, 1)),
         ((1, 1), (0, -1)), ((3, 1),), ((0, 1),))
_FIRST, _LAST = (4, 2, 1, 2), (6, 4, 3, 5)


def _acc(c, v, s):
    if c is None:
        return v if s > 0 else -v
    return c + v if s > 0 else c - v


def _sub(outer, inner):
    return 2 * (outer // 2) + inner // 2, 2 * (outer % 2) + inner % 2


def _forms2(t, get):
    x = []
    for ab in range(4):
        v = None
        for big, s in _FORM[t]:
            v = _acc(v, get(*_sub(big, ab)), s)
        x.append(v)
    return _forms(*x)


def _strassen(prod, emit, init=None):
    c = [None] * 4
    for i in _ORDER:
        m = prod(i)
        for b, s in _INTO[i]:
            if init is not None and _FIRST[b] == i:
                c[b] = init(b)
            c[b] = _acc(c[b], m, s)
            if _LAST[b] == i:
                emit(b, c[b])
        yield


def _strassen2(prod, rmw):
    for t in _ORDER:
        def emit(ab, v):
            for big, s in _INTO[t]:
                rmw(*_sub(big, ab), v, s, _FIRST[big] == t, _LAST[big] == t)
        yield from _strassen(lambda u: prod(7 * t + u), emit)


def _mix(*streams):
    ev = sorted(((k + 0.5) / n, i) for i, (_, n) in enumerate(streams) for k in range(n))
    for _, i in ev:
        next(streams[i][0])
    for g, _ in streams:
        assert next(g, "end") == "end"


def _loop(n, body, unroll=1):
    if unroll == n:
        for i in range(n):
            body(i)
        return

    def step(i, c):
        for u in range(unroll):
            body(i * unroll + u)
        return c
    jax.lax.fori_loop(0, n // unroll, step, 0)


def _al(i, n, m=None):
    return pl.ds(i * n if isinstance(i, int) else pl.multiple_of(i * n, m or n), n)


def _tile(t):
    return _al(t, 128)


def _pk(v):
    return pltpu.bitcast(v.astype(bf16), u32)


def _up(v):
    return pltpu.bitcast(v, bf16)


def _pack2(a, b):
    return pltpu.bitcast(a.astype(f32), u32) | (pltpu.bitcast(b.astype(f32), u32) >> 16)


def _unpack2(w):
    return pltpu.bitcast(w & jnp.uint32(0xFFFF0000), f32), pltpu.bitcast(w << 16, f32)


def _stats(x):
    m = jnp.mean(x, axis=0, keepdims=True)
    xc = x - m
    return xc, m, jax.lax.rsqrt(jnp.mean(xc * xc, axis=0, keepdims=True) + EPS)


def _ln_bwd(dn, n, rstd):
    return (dn - jnp.mean(dn, axis=0, keepdims=True)
            - n * jnp.mean(dn * n, axis=0, keepdims=True)) * rstd


NWT = 4 * 72
NXF, NXT = 14 * 64, 49 * 72
RH = R // 2


def _kernel(x_h, g_h, wr_h, wi_h, ce_h, co_h, cet_h, cot_h, gm_h, wg_h, wu_h, wd_h,
            out_h, dx_h, dwr_h, dwi_h, dwg_h, dwu_h, dwd_h,
            x_s, g_s, ce_s, co_s, cet_s, cot_s, gm_s, wp, xf_s, hn_s, st_s, oacc, dacc,
            xF, xt, xTF, WB, WT, w_s, dws, f, sems):
    copy = pltpu.make_async_copy
    sem_ids = iter(range(64))
    cp = lambda a, b: copy(a, b, sems.at[next(sem_ids)])
    s_g = [sems.at[next(sem_ids)] for _ in range(NG)]
    i_ = next(sem_ids)
    g_in = [copy(g_h.at[:, _tile(t)], g_s.at[t], sems.at[i_]) for t in range(16)]
    c_in = [cp(a, b) for a, b in ((ce_h, ce_s), (co_h, co_s), (gm_h, gm_s), (cet_h, cet_s), (cot_h, cot_s))]
    s_wi, s_r, s_o, s_x = [sems.at[next(sem_ids)] for _ in range(4)]
    s_dw = [sems.at[next(sem_ids)] for _ in range(3)]
    w_in = lambda k, c: copy((wg_h, wu_h, wd_h)[k].at[:, _al(c, BF)], w_s, s_wi)

    dw_out = lambda c: [copy(dws.at[k], h.at[:, _al(c, BF)], s_dw[k])
                        for k, h in enumerate((dwg_h, dwu_h, dwd_h))]

    def row_scale():
        rows = jax.lax.broadcasted_iota(jnp.int32, (R, 128), 0)
        return jnp.where((rows == 0) | (rows == DH // 4), 1.0 / (S * D), 2.0 / (S * D)).astype(f32)

    def dft_d(v, scale, z, c):
        s = (v[:DH] + v[DH:]) * scale
        for r, u in enumerate((s[:Q] + s[Q:], s[:Q] - s[Q:])):
            e = _dot(ce_s[r], u.astype(bf16))
            z[0, _al(r, NE // 2), c] = e[:NE // 2]
            z[1, _al(r, NE // 2), c] = e[NE // 2:]
        o = _dot(co_s[...], ((v[:DH] - v[DH:]) * scale).astype(bf16))
        z[0, NE:, c] = o[:NO]
        z[1, NE:, c] = o[NO:]

    def fft_s(z, zb, sg):
        def fft(i):
            r = _al(i, 16)
            y = _fft16([(z[0, r, _tile(t)], z[1, r, _tile(t)]) for t in range(16)], sg)
            d = zb.at[pl.ds(pl.multiple_of(i * 8, 8), 15 * RH + 8)]
            for t in range(16):
                d[pl.ds(t * RH, 8), :128] = _pk(y[t][0])
                d[pl.ds(t * RH, 8), 128:] = _pk(y[t][1])
        _loop(R // 16, fft)

    def fwd_b(zb, t):
        y = _dot(_up(zb[_al(t, RH, 8), :]), _up(gm_s[_tile(t), :]))
        return y[:, :128], y[:, 128:]

    def adj_b(z, t, yr, yi):
        y = _dot(jnp.concatenate([yr.astype(bf16), yi.astype(bf16)], axis=1), _up(gm_s[_tile(t), :]), NT)
        z[0, :, _tile(t)] = y[:, :128]
        z[1, :, _tile(t)] = y[:, 128:]

    def adj_d(zb, t):
        v = zb.at[pl.ds(t * RH if isinstance(t, int) else pl.multiple_of(t * RH, 8), 2 * RH)]

        def part(r, n):
            return _up(jnp.concatenate([jnp.concatenate([v[pl.ds(a * RH + r, n), _tile(c)] for c in range(2)], axis=0)
                                        for a in range(2)], axis=1))
        e0, e1 = [_dot(cet_s[r], part(r * NE // 4, NE // 4)) for r in range(2)]
        e = jnp.concatenate([e0 + e1, e0 - e1], axis=0)
        o = _dot(cot_s[...], part(NE // 2, NO // 2))
        y = jnp.concatenate([e + o, e - o], axis=0)
        return (t, y[:, :128]), (t + 1, y[:, 128:])

    def x_forms(k, src, g):
        v = src.at[_al(g, 4)]
        d = xTF.at[_al(g, NXT, 8)]
        for t in range(7):
            for o in range(0, Q, 48):
                y = _forms2(t, lambda a, b: v[b, pl.ds(a * Q + o, 48), :].astype(f32))
                for m in range(7):
                    d[pl.ds((7 * t + m) * 72 + o // 2, 24), _tile(k)] = _pk(y[m])
                yield
        d = xF.at[_al(2 * g + k, NXF, 8)]
        for q in range(2):
            for c in range(2):
                y = _forms(*[v[2 * a + q, _tile(2 * b + c), :].astype(f32).T for a in range(2) for b in range(2)])
                for m in range(7):
                    d[_al(2 * m + q, 64), _tile(c)] = _pk(y[m])
                yield
        for q in range(2):
            y = jnp.concatenate([v[2 * q + a, 512:, :].astype(f32) for a in range(2)], axis=0).T
            xt[_al(4 * g + 2 * k + q, 64), :] = _pk(y)
            yield
    NX = 27

    def w_forms_left(i, stage=None):
        st = [r.at[_al(i, NWT, 8)] for r in WT]
        for o in range(0, Q, 16):
            get = lambda a, b: w_s[pl.ds(b * Q + o, 16), _tile(a)].astype(f32)
            if stage:
                for a in range(4):
                    for b in range(4):
                        stage[0][pl.ds((4 * a + b) * Q + o, 16), :] = get(a, b)
                get = lambda a, b: stage[1][pl.ds((4 * a + b) * Q + o, 16), :]
            for t in range(7):
                y = _forms2(t, get)
                for u in range(7):
                    m = _B2A.index(u)
                    st[_B2A.index(t)][pl.ds((m // 2) * 72 + o // 2, 8), _tile(m % 2)] = _pk(y[u])
                yield

    def w_forms_right(i):
        sb = [r.at[_al(i, 128)] for r in WB]
        for c in range(2):
            for o in range(0, 256, 32):
                y = _forms(*[w_s[pl.ds(256 * a + o, 32), _tile(2 * b + c)].astype(f32)
                             for a in range(2) for b in range(2)])
                for m in range(7):
                    sb[m][pl.ds(o // 2, 16), _tile(c)] = _pk(y[_B2A[m]])
                yield
            sb[7][_al(c, 32), :] = _pk(w_s[512:, _al(c, 256)].astype(f32))

    def phase_a(wr_s, wi_s, p0, p1, z, zb):
        x_in = [[copy(x_h.at[:, _tile(4 * g + a)], x_s.at[4 * g + a], s_g[g]) for a in range(4)]
                for g in range(NG)]
        w_c = [copy(wr_h, wr_s, s_r), copy(wi_h, wi_s, s_r)]
        for c in x_in[0] + c_in[:2] + x_in[1] + x_in[2] + x_in[3] + w_c + c_in[2:3] + g_in + c_in[3:]:
            c.start()
        w_in(0, 0).start()

        def clear(t):
            dacc[t] = jnp.zeros((D, 128), f32)
            f[:, t >> 2, t & 3] = jnp.zeros((3, 128, 128), f32)
        _loop(16, clear)
        c_in[0].wait()
        c_in[1].wait()

        def ln1(g):
            for j in range(NG):
                @pl.when(g == j)
                def _():
                    for c in x_in[j]:
                        c.wait()
            for a in range(4):
                t = 4 * g + a
                xc, m, rs = _stats(x_s[t].astype(f32))
                st_s[0, t] = m
                st_s[1, t] = rs
                dft_d(xc, rs, z, _tile(t))

        def wperm(t):
            p0[t, DF - 1:, :] = jnp.zeros((2 * NE - DF + 1, 128), u32)
            p0[t, :DF, :] = _pack2(wr_s[:, _tile(t)], wi_s[:, _tile(t)])
            v = jnp.concatenate([p0[t, pl.ds(0, NE // 2, stride=4), :], p0[t, pl.ds(2, NE // 2, stride=4), :],
                                 p0[t, pl.ds(1, NO, stride=2), :],
                                 jnp.zeros((384 - R, 128), u32)], axis=0).T
            for q in range(3):
                p1[q, _tile(t), :] = v[:, _tile(q)]
        _loop(NG, ln1)
        fft_s(z, zb, -1)
        for c in w_c:
            c.wait()
        _loop(16, wperm, 4)
        c_in[2].wait()
        for c in g_in:
            c.wait()

        def filt(g):
            def f():
                for a in range(4):
                    t = 4 * g + a
                    w = jnp.concatenate([p1[q, pl.ds(t, 128, stride=16), :] for q in range(3)], axis=1).T[:R]
                    wp[t] = w
                    xr, xi = fwd_b(zb, t)
                    xf_s[t] = _pack2(xr.astype(bf16), xi.astype(bf16))
                    yield
                    wr, wi = _unpack2(w)
                    sc = row_scale()
                    adj_b(z, t, (xr * wr - xi * wi) * sc, (xr * wi + xi * wr) * sc)
                    yield
            _mix((f(), 8), (x_forms(1, g_s, g), NX))
        _loop(NG, filt, NG)
        fft_s(z, zb, 1)
        c_in[3].wait()
        c_in[4].wait()

        def ln2_of(g):
            for a in range(0, 4, 2):
                for t, y in adj_d(zb, 4 * g + a):
                    h = x_s[t].astype(f32) + y
                    oacc[t] = h
                    hc, _, rs = _stats(h)
                    hn_s[t] = hc * rs
                    st_s[2, t] = rs
                    yield

        def ln2(g):
            for k in range(3):
                pl.when(g == k)(lambda: w_in(k, 0).wait())
            pl.when(g < 3)(lambda: _mix((chain(w_forms_left(g), w_forms_right(g)), 79)))
            for k in range(3):
                pl.when(g == k)(lambda: w_in((k + 1) % 3, k // 2).start())
            _mix((ln2_of(g), 4))
        _loop(NG, ln2)

    def phase_b(y_s, e, dwacc, w_f):
        def pre_act(slot, g, tick=False):
            wb = [r.at[_al(slot, 384)] for r in WB]
            xf, tl = xF.at[_al(g, 2 * NXF, 8)], xt.at[_al(g, 256)]
            for k in range(3):
                for o in range(2):
                    for q, c in ((0, 0), (1, 1), (0, 1), (1, 0)):
                        def prod(m):
                            return _dot(_up(xf[pl.ds((k // 2) * NXF + (2 * m + q) * 64 + 32 * o, 32), :]),
                                        _up(wb[m][_tile(k), _tile(c)]))

                        def init(b):
                            return _dot(_up(tl[_al(2 * (2 * (k // 2) + b // 2) + o, 32), :])[:, 64 * q:64 * q + 64],
                                        _up(wb[7][pl.ds(k * 128 + 32 * (b % 2), 32), _tile(c)]))

                        def emit(b, v):
                            e[k, 2 * (b // 2) + q, 2 * (b % 2) + c, _al(o, 64)] = v
                            if tick:
                                w_f[_al(32 * k + 16 * q + 8 * c + 4 * o + b, 8), :] = v[:8]
                        yield from _strassen(prod, emit, init)

        def act_block(ev, fv):
            for o in range(0, 128, 32):
                r = pl.ds(o, 32)
                av, u, dp = [ev[k, r, :] for k in range(3)]
                s = 0.5 * jnp.tanh(0.5 * av) + 0.5
                g = av * s
                fv[0, r, :] = dp * u * (s + g * (1.0 - s))
                fv[1, r, :] = dp * g
                fv[2, r, :] = g * u
                yield

        def act():
            for a in range(4):
                for b in range(4):
                    yield from act_block(e.at[:, a, b], f.at[:, a, b])

        def y_forms(fv, yv):
            for k in range(3):
                for t in range(7):
                    for m, v in enumerate(_forms2(t, lambda a, b: fv[k, a, b])):
                        yv[pl.ds((7 * t + m) * 64, 8), _tile(k)] = _pk(v)
                    yield

        def y_view(o):
            al = (lambda v, m: v) if isinstance(o, int) else pl.multiple_of
            return f.at[:, :, :, pl.ds(al(16 * o, 16), 16), :], y_s.at[pl.ds(al(8 * o, 8), 48 * 64 + 8)]

        def y_forms_all():
            for o in range(8):
                yield from y_forms(*y_view(o))

        gy = lambda k, m: _up(y_s[_al(m, 64), _tile(k)])

        def out_dh(slot, g):
            wt = [r.at[_al(slot, 3 * NWT, 8)] for r in WT]
            pr = lambda k, m: _dot(_up(wt[m // 7][pl.ds(k * NWT + (m % 7 // 2) * 72, 72), _tile(m % 7 % 2)]),
                                   gy(k, m), NT)

            def into(ref):
                ref = ref.at[_al(g, 4)]

                def rmw(a, b, v, s, first, last):
                    ref[a, _al(b, Q), :] = _acc(ref[a, _al(b, Q), :], v, s)
                return rmw
            yield from _strassen2(lambda m: pr(2, m), into(oacc))
            yield from _strassen2(lambda m: pr(0, m) + pr(1, m), into(dacc))

        def w_grads(g):
            xv = xTF.at[_al(g, NXT, 8)]
            for k in range(3):
                def rmw(a, b, v, s, first, last):
                    c = dwacc[k, a, b]
                    if first:
                        c = jnp.where(g > 0, c, 0.0)
                    c = _acc(c, v, s)
                    dwacc[k, a, b] = c
                    if last:
                        dws[k, _al(a, Q), _tile(b)] = c.astype(bf16)
                yield from _strassen2(lambda m: _dot(_up(xv[_al(m, 72), _tile(k // 2)]), gy(k, _B2A2[m])), rmw)

        _loop(NG, lambda g: _mix((x_forms(0, hn_s, g), NX)))

        def ffn(nxt):
            it = nxt - 1
            c, g = it >> 2, it & 3
            slot = c & 1
            stage = (w_f.at[pl.ds(96 * 8, 16 * Q)],
                     w_f.at[pl.ds(pl.multiple_of(96 * 8 + 8 * jnp.minimum(nxt, 0), 8), 16 * Q)])
            new_w = (g < 3) & (c < NC - 1)

            @pl.when(new_w)
            def _():
                i = 3 * (1 - slot) + g
                _mix((pre_act(slot, g + 1, True), 168), (y_forms_all(), 168),
                     (w_forms_left(i, stage), 63), (w_forms_right(i), 16))

            @pl.when(jnp.logical_not(new_w) & (nxt < NC * NG))
            def _():
                _mix((pre_act((nxt >> 2) & 1, nxt & 3), 168), (y_forms_all(), 168))

            @pl.when(it == NC * NG - 1)
            def _():
                _loop(8, lambda o: _mix((y_forms(*y_view(o)), 21)))

            @pl.when((g == 0) & (c > 0))
            def _():
                for d in dw_out(c - 1):
                    d.wait()
            nw = [(0, 1, c + 1), (1, 2, c + 1), (2, 0, c + 2)]
            for gg, k, cc in nw:
                pl.when((g == gg) & (cc < NC))(lambda: w_in(k, cc).start())

            @pl.when(it < 0)
            def _():
                _loop(16, lambda i: _mix((act_block(e.at[:, i >> 2, i & 3], f.at[:, i >> 2, i & 3]), 4)), 2)

            @pl.when(it >= 0)
            def _():
                _mix((w_grads(g), 147))
                _mix((out_dh(slot, g), 98), (act(), 64))
            for gg, k, cc in nw:
                pl.when((g == gg) & (cc < NC))(lambda: w_in(k, cc).wait())

            @pl.when((g == NG - 1) & (it >= 0))
            def _():
                for d in dw_out(c):
                    d.start()
        w_in(0, 1).wait()
        _loop(NC * NG + 1, ffn)

    def phase_c(wr_s, wi_s, p0, p1, z, zb):
        o_out = [copy(g_s.at[t], out_h.at[:, _tile(t)], s_o) for t in range(16)]
        x_out = lambda t: copy(x_s.at[t], dx_h.at[:, _tile(t)], s_x)
        w_c = lambda g: [copy(b.at[:, _al(g, 512)], a.at[:, _al(g, 512)], s_r)
                         for a, b in ((dwr_h, wr_s), (dwi_h, wi_s))]

        def ln2b(t):
            dh = g_s[t].astype(f32) + _ln_bwd(dacc[t], hn_s[t], st_s[2, t])
            g_s[t] = oacc[t].astype(bf16)
            dacc[t] = dh
            dft_d(dh, 1.0, z, _tile(t))
        _loop(16, ln2b, 8)
        for c in o_out:
            c.start()
        fft_s(z, zb, -1)

        def filt_b(t):
            yr, yi = fwd_b(zb, t)
            sc = row_scale()
            yr, yi = yr * sc, yi * sc
            wr, wi = _unpack2(wp[t])
            adj_b(z, t, yr * wr + yi * wi, yi * wr - yr * wi)
            xr, xi = _unpack2(xf_s[t])
            v = _pack2((yr * xr + yi * xi).astype(bf16), (yi * xr - yr * xi).astype(bf16))
            v = jnp.concatenate([v, jnp.zeros((384 - R, 128), u32)], axis=0).T
            for q in range(3):
                p1[q, pl.ds(t, 128, stride=16), :] = v[:, _tile(q)]
        _loop(16, filt_b, 16)

        def wperm_b(t):
            v = jnp.concatenate([p1[q, _tile(t), :] for q in range(3)], axis=1).T
            p0[t, pl.ds(0, NE // 2, stride=4), :] = v[:NE // 2]
            p0[t, pl.ds(2, NE // 2, stride=4), :] = v[NE // 2:NE]
            p0[t, pl.ds(1, NO, stride=2), :] = v[NE:R]
            a, b = _unpack2(p0[t, :DF, :])
            wr_s[:, _tile(t)] = a.astype(bf16)
            wi_s[:, _tile(t)] = b.astype(bf16)
        fft_s(z, zb, 1)

        def ln1b(g):
            for a in range(0, 4, 2):
                for t, y in adj_d(zb, 4 * g + a):
                    rs = st_s[1, t]
                    n = (x_s[t].astype(f32) - st_s[0, t]) * rs
                    x_s[t] = (dacc[t] + _ln_bwd(y, n, rs)).astype(bf16)
                    wperm_b(t)
            for c in [x_out(4 * g + a) for a in range(4)] + w_c(g):
                c.start()
        _loop(NG, ln1b)
        for c in dw_out(NC - 1) + o_out + [x_out(t) for t in range(16)] + [c for g in range(NG) for c in w_c(g)]:
            c.wait()

    V = pltpu.VMEM
    spectral = (V((DF, S), bf16), V((DF, S), bf16), V((16, 2 * NE, 128), u32), V((3, S, 128), u32),
                V((2, R, S), f32), V((16 * RH, 256), u32))
    pl.run_scoped(phase_a, *spectral)
    pl.run_scoped(phase_b, V((49 * 64, 384), u32), V((3, 4, 4, 128, 128), f32),
                  V((3, 4, 4, Q, 128), f32), V((96 * 8 + 16 * Q, 128), f32))
    pl.run_scoped(phase_c, *spectral)


@jax.jit
def pallas_sequential_preLN__spectral_gfnet__swiglu_ffn__prompt_kernel(
    A_x: jax.Array,
    A_w_r: jax.Array,
    A_w_i: jax.Array,
    B_x: jax.Array,
    B_w_gate: jax.Array,
    B_w_up: jax.Array,
    B_w_down: jax.Array,
    grad_out: jax.Array,
):
    hbm = pl.BlockSpec(memory_space=pltpu.HBM)
    sds = jax.ShapeDtypeStruct
    V = pltpu.VMEM
    consts = (_CE, _CO, _CET, _COT, _G)
    out, dx, dwr, dwi, dwg, dwu, dwd = pl.pallas_call(
        _kernel,
        in_specs=[hbm] * 12,
        out_specs=[hbm] * 7,
        out_shape=[sds((D, S), bf16)] * 2 + [sds((DF, S), bf16)] * 2 + [sds((D, F), bf16)] * 3,
        scratch_shapes=[V((16, D, 128), bf16)] * 2 + [V(c.shape, c.dtype) for c in consts]
        + [V((16, R, 128), u32)] * 2 + [V((16, D, 128), f32), V((4, 16, 1, 128), f32)]
        + [V((16, D, 128), f32)] * 2
        + [V((2 * NG * NXF, 256), u32), V((NG * 256, 128), u32), V((NG * NXT, 256), u32),
           [V((6 * 128, 256), u32)] * 8, [V((6 * NWT, 256), u32)] * 7, V((D, BF), bf16),
           V((3, D, BF), bf16), V((3, 4, 4, 128, 128), f32), pltpu.SemaphoreType.DMA((17,))],
        compiler_params=pltpu.CompilerParams(vmem_limit_bytes=120 * 2**20),
    )(A_x.reshape(S, D).T, grad_out.reshape(S, D).T, A_w_r.T, A_w_i.T, *consts,
      B_w_gate, B_w_up, B_w_down.T)
    return (out.T.reshape(1, S, D), dx.T.reshape(1, S, D), dwr.T, dwi.T, dwg, dwu, dwd.T)
```
